```python
import os as _os
_os.environ.setdefault("JAX_PLATFORMS", "cpu")
import jax
import jax.numpy as jnp

def _softmax(x, axis=-1):
    return jax.nn.softmax(x, axis=axis)
def _gelu(x):
    return jax.nn.gelu(x, approximate=True)
def _silu(x):
    return jax.nn.silu(x)
def _sigmoid(x):
    return jax.nn.sigmoid(x)
def _layernorm(x, axis=-1, eps=1e-5):
    m = jnp.mean(x, axis=axis, keepdims=True)
    v = jnp.var(x, axis=axis, keepdims=True)
    return (x - m) / jnp.sqrt(v + eps)
def _scatter_add(tgt, idx, src, axis=0):
    return tgt.at[idx].add(src)
def _segment_sum(src, seg, n):
    return jax.ops.segment_sum(src, seg, n)
class _Rng:
    def __init__(self, key):
        self._k = key
    def _next(self):
        self._k, sub = jax.random.split(self._k)
        return sub
    def normal(self, shape):
        return jax.random.normal(self._next(), shape, dtype=jnp.bfloat16)
    def randint(self, lo, hi, shape):
        return jax.random.randint(self._next(), shape, lo, hi, dtype=jnp.int32)
    def uniform(self, shape, lo=0.0, hi=1.0):
        return jax.random.uniform(self._next(), shape, jnp.bfloat16, lo, hi)
    def permutation(self, n):
        return jax.random.permutation(self._next(), n)


kernel_name = 'gated_mix__linear_attn_block__sliding_local_dilated__prompt'

def setup_inputs():
    _rng = _Rng(jax.random.key(int.from_bytes(__import__("os").urandom(4), "little")))
    _w = (lambda a: (lambda t: t.astype(jnp.bfloat16) if jnp.issubdtype(t.dtype, jnp.floating) else t)(jnp.asarray(a)))
    def _A_setup():
        B, S, D = 1, 2048, 512
        return {
            "x": _w((lambda *s: _rng.normal(s) * 0.05)(B, S, D)),
            "wqkv": _w((lambda *s: _rng.normal(s) * 1.6)(D, 3 * D)),
            "wo": _w((lambda *s: _rng.normal(s) * 0.8)(D, D)),
        }
    _A_in = _A_setup()

    def _B_setup():
        B, S, D = 1, 2048, 512
        return {
            "x": _w((lambda *s: _rng.normal(s) * 0.05)(B, S, D)),
            "wqkv": _w((lambda *s: _rng.normal(s) * 0.8)(D, 3 * D)),
            "wo": _w((lambda *s: _rng.normal(s) * 0.05)(D, D)),
        }
    _B_in = _B_setup()

    return {
        "A_x": _A_in["x"],
        "A_wqkv": _A_in["wqkv"],
        "A_wo": _A_in["wo"],
        "B_x": _B_in["x"],
        "B_wqkv": _B_in["wqkv"],
        "B_wo": _B_in["wo"],
        "gate_w": _w((lambda *s: _rng.normal(s) * 0.05)(512) * 16.0),
    }

def reference(A_x, A_wqkv, A_wo, B_x, B_wqkv, B_wo, gate_w):
    def _A_ref(x, wqkv, wo):
        B, S, D = x.shape
        H = 32; Dh = D // H
        qkv = (lambda x, *d: x.transpose(*d))((x @ wqkv).reshape(B, S, 3, H, Dh), 2, 0, 3, 1, 4)
        q, k, v = qkv[0], qkv[1], qkv[2]
        phi = lambda t: jnp.where(t > 0, t + 1, jnp.exp(t)) + 1e-6
        pq, pk = phi(q), phi(k)
        kv = jnp.einsum("bhsd,bhse->bhde", pk, v)
        z = jnp.einsum("bhsd->bhd", pk)
        num = jnp.einsum("bhqd,bhde->bhqe", pq, kv)
        den = jnp.einsum("bhqd,bhd->bhq", pq, z)[..., None] + 1e-6
        o = num / den
        return (lambda x, *d: x.transpose(*d))(o, 0, 2, 1, 3).reshape(B, S, D) @ wo

    def _B_ref(x, wqkv, wo):
        B, S, D = x.shape
        H = 32; Dh = D // H
        W, dil = 8, 2
        qkv = (lambda x, *d: x.transpose(*d))((x @ wqkv).reshape(B, S, 3, H, Dh), 2, 0, 3, 1, 4)
        q, k, v = qkv[0], qkv[1], qkv[2]
        scale = Dh ** -0.5
        pos = jnp.arange(S)
        off = jnp.arange(W) * dil
        idx = pos[:, None] - off[None, :]
        mask = idx >= 0
        idx_c = jnp.where(mask, idx, 0).reshape(-1)
        kg = k[:, :, idx_c, :].reshape(B, H, S, W, Dh)
        vg = v[:, :, idx_c, :].reshape(B, H, S, W, Dh)
        logits = jnp.einsum("bhsd,bhswd->bhsw", q, kg) * scale
        logits = jnp.where(mask[None, None, :, :], logits, -1e9)
        attn = _softmax(logits, axis=-1)
        o = jnp.einsum("bhsw,bhswd->bhsd", attn, vg)
        return (lambda x, *d: x.transpose(*d))(o, 0, 2, 1, 3).reshape(B, S, D) @ wo

    x = A_x
    g = _sigmoid((x * gate_w).sum(-1, keepdims=True))
    a = _A_ref(x, A_wqkv, A_wo)
    b = _B_ref(x, B_wqkv, B_wo)
    return g * a + (1 - g) * b
```

```python
import jax
import jax.numpy as jnp
from jax import lax
from jax.experimental import pallas as pl
from jax.experimental.pallas import tpu as pltpu

S, D = 2048, 512
NG = 4
NC = 8
CW = 256
WIN = 8
F32, BF16, U32 = jnp.float32, jnp.bfloat16, jnp.uint32
NT = (((1,), (1,)), ((), ()))
NN = (((1,), (0,)), ((), ()))


def _dot(a, b, dims=NN):
    return lax.dot_general(a, b, dims, preferred_element_type=F32)


def _phi(t):
    return jnp.where(t > 0, t + 1.0, jnp.exp(t)) + 1e-6


def _kernel(xa_h, wa_h, woa_h, wb_h, wob_h, gw_ref, out_h,
            xraw, xa, wa, wb, woa, wob, wt, wfin,
            kx0, kx1, vx0, vx1, qb0, qb1, pq0, pq1, pk, zacc, zb, gate, o_scr, obuf, sems):
    def xcopy(src, j, c):
        return pltpu.make_async_copy(src.at[:, pl.ds(c * 128, 128)], xraw.at[j, c], sems.at[j * 4 + c])
    cp_wb = pltpu.make_async_copy(wb_h, wb, sems.at[8])
    cp_wa = pltpu.make_async_copy(wa_h, wa, sems.at[9])
    cp_woa = pltpu.make_async_copy(woa_h, woa, sems.at[10])
    cp_wob = pltpu.make_async_copy(wob_h, wob, sems.at[11])
    cp_wb.start()
    for c in range(4):
        xcopy(xa_h, 0, c).start()
    cp_wa.start()
    cp_wob.start()
    cp_woa.start()

    kx, vx, qb, pq = (kx0, kx1), (vx0, vx1), (qb0, qb1), (pq0, pq1)
    r_i = lax.broadcasted_iota(jnp.int32, (128, 128), 0)
    f_i = lax.broadcasted_iota(jnp.int32, (128, 128), 1)
    perm = jnp.where(f_i == (r_i % 8) * 16 + r_i // 8, 1.0, 0.0).astype(BF16)

    def permute_x(j, dst):
        for c in range(4):
            src = xraw.at[j, c].bitcast(U32)
            for t in range(NC):
                dst[t * 128:(t + 1) * 128, c * 128:(c + 1) * 128] = src[pl.ds(t, 128, stride=8), :]

    cp_wb.wait()
    for g in range(NG):
        for j in range(3):
            col = j * D + g * 128
            wt[g, j * 64:(j + 1) * 64, :] = pltpu.bitcast(_dot(perm, wb[:, col:col + 128], NT).astype(BF16), U32)
    for c in range(4):
        xcopy(xa_h, 0, c).wait()
    permute_x(0, xa)
    cp_wa.wait()
    for g in range(NG):
        for j in range(2):
            col = j * D + g * 128
            wt[g, 192 + j * 64:192 + (j + 1) * 64, :] = pltpu.bitcast(_dot(perm, wa[:, col:col + 128], NT).astype(BF16), U32)
        wt[g, 320:328, :] = pltpu.bitcast(jnp.broadcast_to(gw_ref[...].reshape(1, D), (16, D)), U32)

    lane = lax.broadcasted_iota(jnp.int32, (128, 128), 1)
    lane8 = lax.broadcasted_iota(jnp.int32, (8, CW), 1)

    def shifted(a):
        r0 = pltpu.roll(a[:, :128], 2, 1)
        r1 = pltpu.roll(a[:, 128:], 2, 1)
        return jnp.concatenate([jnp.where(lane < 2, 0.0, r0), jnp.where(lane < 2, r0, r1)], axis=1)

    def rows(t):
        return pl.ds(pl.multiple_of(t * CW, CW), CW)

    def proj_steps(g, t, first):
        par = g % 2
        def mm(w):
            xs = pltpu.bitcast(xa[pl.ds(pl.multiple_of(t * 128, 128), 128), :], BF16)
            return _dot(pltpu.bitcast(w, BF16), xs, NT)
        def s_q():
            qb[par][t] = mm(wt[g, pl.ds(pl.multiple_of(0 + (t // 8) * 8, 8), 64), :]) * 0.25
        def s_k():
            k = mm(wt[g, pl.ds(pl.multiple_of(64 + (t // 8) * 8, 8), 64), :])
            kx[par][t + 8] = k
            kx[par][t] = shifted(k)
        def s_v():
            v = mm(wt[g, pl.ds(pl.multiple_of(128 + (t // 8) * 8, 8), 64), :])
            vx[par][t + 8] = v
            vx[par][t] = shifted(v)
        def s_pq():
            pq[par][t] = _phi(mm(wt[g, pl.ds(pl.multiple_of(192 + (t // 8) * 8, 8), 64), :]))
        def s_pk():
            if first:
                ra = mm(wt[g, pl.ds(pl.multiple_of(256 + (t // 8) * 8, 8), 72), :])
                gate[t] = jax.nn.sigmoid(ra[128:136])
                ra = ra[0:128]
            else:
                ra = mm(wt[g, pl.ds(pl.multiple_of(256 + (t // 8) * 8, 8), 64), :])
            pkv = _phi(ra)
            pk[t, g * 128:(g + 1) * 128, :] = pkv.astype(BF16)
            zacc[...] += pkv[:, :128] + pkv[:, 128:]
        return [s_k, s_v, s_pk, s_pq, s_q]

    def proj(g, t, first):
        for f in proj_steps(g, t, first):
            f()

    def finish_z():
        zb[...] = jnp.broadcast_to(jnp.sum(zacc[...], axis=1, keepdims=True), (128, CW))
        zacc[...] = jnp.zeros_like(zacc)

    def put_o(blk, t, val):
        vt = val.T.astype(BF16)
        for h in range(2):
            o_scr[blk, pl.ds(pl.multiple_of(h * 1024 + t * 128, 128), 128), :] = vt[h * 128:(h + 1) * 128]

    def attend_steps(g, t):
        par = g % 2
        st = {}
        def s_norm():
            gt = gate[t]
            den = None
            for d in range(16):
                sl = slice(8 * d, 8 * d + 8)
                term = pq[par][t, sl, :] * zb[sl, :]
                den = term if den is None else den + term
            sc = gt / (den + 1e-6)
            put_o(g, t, jnp.concatenate([pq[par][t, 8 * d:8 * d + 8, :] * sc for d in range(16)], axis=0))
        def s_logit(d0, d1):
            lg = st.setdefault("lg", [None] * WIN)
            for d in range(d0, d1):
                sl = slice(8 * d, 8 * d + 8)
                qd = qb[par][t, sl, :]
                for w in range(WIN):
                    term = qd * kx[par][t + 8 - w, sl, :]
                    lg[w] = term if lg[w] is None else lg[w] + term
        def s_soft():
            lg = st["lg"]
            for w in range(1, WIN):
                lg[w] = jnp.where(lane8 < jnp.where(t < w, 2, 0), -1e9, lg[w])
            m = lg[0]
            for w in range(1, WIN):
                m = jnp.maximum(m, lg[w])
            p = [jnp.exp(l - m) for l in lg]
            tot = p[0]
            for w in range(1, WIN):
                tot = tot + p[w]
            sc = (1.0 - gate[t]) / tot
            st["p"] = [x * sc for x in p]
            st["o"] = []
        def s_pv(d0, d1):
            p = st["p"]
            for d in range(d0, d1):
                sl = slice(8 * d, 8 * d + 8)
                acc = None
                for w in range(WIN):
                    term = p[w] * vx[par][t + 8 - w, sl, :]
                    acc = term if acc is None else acc + term
                st["o"].append(acc)
        def s_put():
            put_o(NG + g, t, jnp.concatenate(st["o"], axis=0))
        def tie(v):
            if g + 1 >= NG: return
            wt[g + 1, pl.ds(pl.multiple_of(328 + 8 * t, 8), 8), 0:128] = pltpu.bitcast(v[0:8, 0:128], U32)
        return [lambda: (s_logit(0, 8)), lambda: (s_logit(8, 16), s_soft(), tie(st["p"][7])),
                lambda: (s_pv(0, 8)),
                lambda: (s_pv(8, 16), s_put()), s_norm]

    def attend(g, t):
        for f in attend_steps(g, t):
            f()

    def loop(body):
        lax.fori_loop(0, NC, lambda t, c: (body(t), c)[1], 0, unroll=2)

    zacc[...] = jnp.zeros_like(zacc)
    loop(lambda t: proj(0, t, True))
    finish_z()

    def stage(g, c):
        def body(t):
            for f1, f2 in zip(proj_steps(g, t, False), attend_steps(g - 1, t)):
                f1()
                f2()
        loop(body)
        finish_z()
        return c
    for g_ in range(1, NG):
        stage(g_, 0)

    cp_wob.wait()
    cp_woa.wait()
    for g in range(NG):
        wfin[D + g * 128:D + (g + 1) * 128, :] = _dot(perm, wob[g * 128:(g + 1) * 128, :]).astype(BF16)

    gacc = qb0

    def body_last(t):
        attend(NG - 1, t)
        half = t // 4
        cb = t % 4
        acc = None
        for tt in range(NC):
            term = _dot(pk[tt, pl.ds(pl.multiple_of(cb * 128, 128), 128), :],
                        pltpu.bitcast(xa[tt * 128:(tt + 1) * 128, pl.ds(pl.multiple_of(half * CW, CW), CW)], BF16))
            acc = term if acc is None else acc + term
        gacc[t] = acc
    loop(body_last)

    hmask = (r_i % 8) == (f_i // 16)
    for g in range(NG):
        gg = jnp.concatenate([gacc[g], gacc[4 + g]], axis=1).astype(BF16)
        kv = _dot(gg, wa[:, 2 * D + g * 128:2 * D + (g + 1) * 128])
        kv = jnp.where(hmask, kv, 0.0).astype(BF16)
        wfin[g * 128:(g + 1) * 128, :] = _dot(kv, woa[g * 128:(g + 1) * 128, :]).astype(BF16)

    def ocopy(h, c):
        return pltpu.make_async_copy(obuf.at[c, pl.ds(h * 1024, 1024), :],
                                     out_h.at[pl.ds(h * 1024, 1024), pl.ds(c * 128, 128)],
                                     sems.at[12 + h * 4 + c])
    for h in range(2):
        for n in range(2):
            for q4 in range(2):
                r0 = h * 1024 + q4 * 512
                lhs = jnp.concatenate([o_scr[b, r0:r0 + 512, :] for b in range(2 * NG)], axis=1)
                res = _dot(lhs, wfin[:, n * 256:(n + 1) * 256]).astype(BF16)
                for cc in range(2):
                    dst = obuf.at[n * 2 + cc].bitcast(U32)
                    for tt in range(4):
                        t = q4 * 4 + tt
                        dst[pl.ds(h * 512 + t, 64, stride=8), :] = pltpu.bitcast(
                            res[tt * 128:(tt + 1) * 128, cc * 128:(cc + 1) * 128], U32)
            for cc in range(2):
                ocopy(h, n * 2 + cc).start()
    for h in range(2):
        for c in range(4):
            ocopy(h, c).wait()


@jax.jit
def pallas_gated_mix__linear_attn_block__sliding_local_dilated__prompt_kernel(
    A_x, A_wqkv, A_wo, B_x, B_wqkv, B_wo, gate_w,
):
    V = pltpu.VMEM
    hbm = pl.BlockSpec(memory_space=pl.ANY)
    out = pl.pallas_call(
        _kernel,
        out_shape=jax.ShapeDtypeStruct((S, D), BF16),
        in_specs=[hbm] * 5 + [pl.BlockSpec(memory_space=V)],
        out_specs=hbm,
        scratch_shapes=[
            V((1, 4, S, 128), BF16),
            V((S // 2, D), U32),
            V((D, 3 * D), BF16), V((D, 3 * D), BF16),
            V((D, D), BF16), V((D, D), BF16),
            V((NG, 328 + 64, D), U32),
            V((2 * D, D), BF16),
            *[V((16, 128, CW), F32)] * 4,
            *[V((NC, 128, CW), F32)] * 4,
            V((NC, D, CW), BF16),
            V((128, 128), F32), V((128, CW), F32),
            V((NC, 8, CW), F32),
            V((2 * NG, S, 128), BF16),
            V((4, S, 128), BF16),
            pltpu.SemaphoreType.DMA((20,)),
        ],
        compiler_params=pltpu.CompilerParams(vmem_limit_bytes=100 * 2**20),
        name="gated_mix",
    )(A_x.reshape(S, D), A_wqkv, A_wo, B_wqkv, B_wo, gate_w)
    return out.reshape(1, S, D)
```
